```python
import os as _os
_os.environ.setdefault("JAX_PLATFORMS", "cpu")
import jax
import jax.numpy as jnp

def _softmax(x, axis=-1):
    return jax.nn.softmax(x, axis=axis)
def _gelu(x):
    return jax.nn.gelu(x, approximate=True)
def _silu(x):
    return jax.nn.silu(x)
def _sigmoid(x):
    return jax.nn.sigmoid(x)
def _layernorm(x, axis=-1, eps=1e-5):
    m = jnp.mean(x, axis=axis, keepdims=True)
    v = jnp.var(x, axis=axis, keepdims=True)
    return (x - m) / jnp.sqrt(v + eps)
def _scatter_add(tgt, idx, src, axis=0):
    return tgt.at[idx].add(src)
def _segment_sum(src, seg, n):
    return jax.ops.segment_sum(src, seg, n)
class _Rng:
    def __init__(self, key):
        self._k = key
    def _next(self):
        self._k, sub = jax.random.split(self._k)
        return sub
    def normal(self, shape):
        return jax.random.normal(self._next(), shape, dtype=jnp.bfloat16)
    def randint(self, lo, hi, shape):
        return jax.random.randint(self._next(), shape, lo, hi, dtype=jnp.int32)
    def uniform(self, shape, lo=0.0, hi=1.0):
        return jax.random.uniform(self._next(), shape, jnp.bfloat16, lo, hi)
    def permutation(self, n):
        return jax.random.permutation(self._next(), n)


kernel_name = 'gated_mix__sliding_block__sliding_local_dilated__prompt'

def setup_inputs():
    _rng = _Rng(jax.random.key(int.from_bytes(__import__("os").urandom(4), "little")))
    _w = (lambda a: (lambda t: t.astype(jnp.bfloat16) if jnp.issubdtype(t.dtype, jnp.floating) else t)(jnp.asarray(a)))
    def _A_setup():
        B, S, D = 1, 2048, 640
        return {
            "x": _w((lambda *s: _rng.normal(s) * 0.05)(B, S, D)),
            "wqkv": _w((lambda *s: _rng.normal(s) * 0.8)(D, 3 * D)),
            "wo": _w((lambda *s: _rng.normal(s) * 0.05)(D, D)),
        }
    _A_in = _A_setup()

    def _B_setup():
        B, S, D = 1, 2048, 640
        return {
            "x": _w((lambda *s: _rng.normal(s) * 0.05)(B, S, D)),
            "wqkv": _w((lambda *s: _rng.normal(s) * 0.8)(D, 3 * D)),
            "wo": _w((lambda *s: _rng.normal(s) * 0.05)(D, D)),
        }
    _B_in = _B_setup()

    return {
        "A_x": _A_in["x"],
        "A_wqkv": _A_in["wqkv"],
        "A_wo": _A_in["wo"],
        "B_x": _B_in["x"],
        "B_wqkv": _B_in["wqkv"],
        "B_wo": _B_in["wo"],
        "gate_w": _w((lambda *s: _rng.normal(s) * 0.05)(640) * 16.0),
    }

def reference(A_x, A_wqkv, A_wo, B_x, B_wqkv, B_wo, gate_w):
    def _A_ref(x, wqkv, wo):
        B, S, D = x.shape
        H = 32; Dh = D // H; W = 256
        qkv = (lambda x, *d: x.transpose(*d))((x @ wqkv).reshape(B, S, 3, H, Dh), 2, 0, 3, 1, 4)
        q, k, v = qkv[0], qkv[1], qkv[2]
        scores = jnp.einsum("bhqd,bhkd->bhqk", q, k) * (Dh ** -0.5)
        idx = jnp.arange(S)
        mask = (idx[:, None] - idx[None, :] >= 0) & (idx[:, None] - idx[None, :] < W)
        scores = jnp.where(mask[None, None], scores, -1e9)
        p = _softmax(scores, axis=-1)
        o = jnp.einsum("bhqk,bhkd->bhqd", p, v)
        return (lambda x, *d: x.transpose(*d))(o, 0, 2, 1, 3).reshape(B, S, D) @ wo

    def _B_ref(x, wqkv, wo):
        B, S, D = x.shape
        H = 32; Dh = D // H
        W, dil = 8, 2
        qkv = (lambda x, *d: x.transpose(*d))((x @ wqkv).reshape(B, S, 3, H, Dh), 2, 0, 3, 1, 4)
        q, k, v = qkv[0], qkv[1], qkv[2]
        scale = Dh ** -0.5
        pos = jnp.arange(S)
        off = jnp.arange(W) * dil
        idx = pos[:, None] - off[None, :]
        mask = idx >= 0
        idx_c = jnp.where(mask, idx, 0).reshape(-1)
        kg = k[:, :, idx_c, :].reshape(B, H, S, W, Dh)
        vg = v[:, :, idx_c, :].reshape(B, H, S, W, Dh)
        logits = jnp.einsum("bhsd,bhswd->bhsw", q, kg) * scale
        logits = jnp.where(mask[None, None, :, :], logits, -1e9)
        attn = _softmax(logits, axis=-1)
        o = jnp.einsum("bhsw,bhswd->bhsd", attn, vg)
        return (lambda x, *d: x.transpose(*d))(o, 0, 2, 1, 3).reshape(B, S, D) @ wo

    x = A_x
    g = _sigmoid((x * gate_w).sum(-1, keepdims=True))
    a = _A_ref(x, A_wqkv, A_wo)
    b = _B_ref(x, B_wqkv, B_wo)
    return g * a + (1 - g) * b
```

```python
import functools
import jax
import jax.numpy as jnp
import numpy as np
import jax.experimental.pallas as pl
import jax.experimental.pallas.tpu as pltpu

S, D, H, DH = 2048, 640, 32, 20
TQ = 128
NB = S // TQ
NPAIR = 16
RA = 320
RB = 80
PADA, PADB = 256, 16
NEG = -1e30
NT = (((1,), (1,)), ((), ()))
F32, BF16 = jnp.float32, jnp.bfloat16
MODES = ['']
DEPTH = (2, 2)
ORDER = 'pqePQfsS'
EOFF = 0
VJ = 2
OJ = [(128 * c, 128 * c + 128) for c in range(5)]
OSTEP = 2

def _pair_tile(p):
    lo, hi = 40 * p, 40 * p + 39
    if lo // 128 == hi // 128:
        return (lo // 128, lo - 128 * (lo // 128))
    lo2, hi2 = lo - 64, hi - 64
    assert lo2 // 128 == hi2 // 128
    return (5 + lo2 // 128, lo2 - 128 * (lo2 // 128))
PT = [_pair_tile(p) for p in range(NPAIR)]
SC = (DH ** -0.5) * float(np.log2(np.e))


def kernel(x_hbm, wa_hbm, woa_hbm, wb_hbm, wob_hbm, gw_ref, o_ref,
           xs_ref, w_ref, wo_st, wvt_ref, wot_ref, q_ref, ka_ref, va_ref, kb_ref, vb_ref, g_ref, bias_ref, ot_ref, sems):
    i = pl.program_id(0)
    q0 = i * TQ
    cat1 = lambda xs: jnp.concatenate(xs, axis=1)

    def copies():
        cs = {}
        cs['x'] = [pltpu.make_async_copy(x_hbm.at[0:256], xs_ref.at[0:256], sems.at[0])]
        cs['x1'] = [pltpu.make_async_copy(x_hbm.at[256:S], xs_ref.at[256:S], sems.at[6])]
        for bi, w_hbm in enumerate((wa_hbm, wb_hbm)):
            cs['qk%d' % bi] = [pltpu.make_async_copy(w_hbm.at[:, 0:2 * D], w_ref.at[bi, :, 0:2 * D], sems.at[1 + 2 * bi])]
            cs['v%d' % bi] = [pltpu.make_async_copy(w_hbm.at[:, 2 * D:3 * D], w_ref.at[bi, :, 2 * D:3 * D], sems.at[2 + 2 * bi])]
        cs['wo'] = [pltpu.make_async_copy(w, wo_st.at[bi], sems.at[5]) for bi, w in enumerate((woa_hbm, wob_hbm))]
        return cs

    def wait(cs, name):
        for c in cs[name]:
            c.wait()

    def shifted(tiles):
        lane = jax.lax.broadcasted_iota(jnp.int32, tiles[0].shape, 1)
        r = [pltpu.roll(t, 64, 1) for t in tiles]
        return [jnp.where(lane < 64, r[t], r[t + 1]) for t in range(4)]

    def xblk(blk):
        return xs_ref[pl.ds(pl.multiple_of(blk * TQ, TQ), TQ), :]

    def proj_jobs(blk):
        jobs = []
        carry = {}
        lane = jax.lax.broadcasted_iota(jnp.int32, (TQ, 128), 1)

        def qk_job(bi, part, t):
            def f():
                y = jnp.dot(xblk(blk), w_ref[bi, :, 128 * (5 * part + t):128 * (5 * part + t + 1)], preferred_element_type=F32)
                if part == 0:
                    y = y * SC
                r = pltpu.roll(y, 64, 1)
                outs = [(t, y)]
                if t > 0:
                    outs.append((4 + t, jnp.where(lane < 64, carry[(bi, part)], r)))
                carry[(bi, part)] = r
                for tt, val in outs:
                    if part == 0:
                        q_ref[blk % 2, bi, tt] = val.astype(BF16)
                    else:
                        k_ref, pad = ((ka_ref, PADA), (kb_ref, PADB))[bi]
                        k_ref[tt, pl.ds(pl.multiple_of(blk * TQ + pad, 16), TQ), :] = val.astype(BF16)
            return f

        def v_job(bi, c):
            def f():
                ch = D // VJ
                gate = (c == VJ - 1 and bi == 0)
                n = ch + 16 if gate else ch
                w = cat1([wvt_ref[bi, t, ch * c:ch * c + n, :] for t in range(5)])
                vt = jax.lax.dot_general(w, xblk(blk), NT, preferred_element_type=F32)
                ones8 = jnp.ones((8, TQ), F32)
                v_ref = (va_ref, vb_ref)[bi]
                kt = blk + (2, 1)[bi]
                for pp in range(NPAIR // VJ):
                    v_ref[(NPAIR // VJ) * c + pp, kt] = jnp.concatenate([vt[40 * pp:40 * pp + 40], ones8], axis=0).astype(BF16)
                if gate:
                    g_ref[blk % 2] = jax.nn.sigmoid(vt[ch:ch + 8])
            return f
        for bi in range(2):
            for part in range(2):
                for t in range(5):
                    jobs.append(qk_job(bi, part, t))
            for c in range(VJ):
                jobs.append(v_job(bi, c))
        return jobs

    def out_jobs(oslot):
        st = {}
        def tr(lo, hi):
            def f():
                for t in range(lo, hi):
                    st[t] = ot_ref[oslot, 128 * t:128 * t + 128, :].T.astype(BF16)
            return f
        def job(t):
            def f():
                o = cat1([st[k] for k in range(10)])
                w = jnp.concatenate([wo_st[0, :, 128 * t:128 * t + 128], wo_st[1, :, 128 * t:128 * t + 128]], axis=0)
                o_ref[:, 128 * t:128 * t + 128] = jnp.dot(o, w, preferred_element_type=F32).astype(BF16)
            return f
        return [tr(0, 5), tr(5, 10)] + [job(t) for t in range(5)]

    @pl.when(i == 0)
    def _init():
        cs = copies()
        for name in ('x', 'qk0', 'v0', 'qk1', 'v1', 'wo', 'x1'):
            for c in cs[name]:
                c.start()
        gw = jnp.broadcast_to(gw_ref[...], (16, D))
        for bi in range(2):
            for t in range(5):
                wvt_ref[bi, t, D:D + 16, :] = gw[:, 128 * t:128 * t + 128]
        ka_ref[:, 0:PADA, :] = jnp.zeros((9, PADA, 128), BF16)
        va_ref[:, 0:2] = jnp.zeros((NPAIR, 2, 48, 128), BF16)
        kb_ref[:, 0:PADB, :] = jnp.zeros((9, PADB, 128), BF16)
        vb_ref[:, 0:1] = jnp.zeros((NPAIR, 1, 48, 128), BF16)
        r = jax.lax.broadcasted_iota(jnp.int32, (RB, 128), 0)
        c = jax.lax.broadcasted_iota(jnp.int32, (RB, 128), 1) & 63
        d = 16 + c - r
        valid = (d >= 0) & (d < 16) & ((d & 1) == 0)
        bias_ref[0] = jnp.where(valid & (r >= 16), 0.0, NEG)
        bias_ref[1] = jnp.where(valid, 0.0, NEG)
        wait(cs, 'x')
        jobs = proj_jobs(0)
        for bi in range(2):
            wait(cs, 'qk%d' % bi)
            for j in jobs[(10 + VJ) * bi:(10 + VJ) * bi + 10]:
                j()
            wait(cs, 'v%d' % bi)
            for kt in range(5):
                for nt in range(5):
                    wvt_ref[bi, kt, 128 * nt:128 * nt + 128, :] = w_ref[bi, 128 * kt:128 * kt + 128, 2 * D + 128 * nt:2 * D + 128 * nt + 128].T
            for j in jobs[(10 + VJ) * bi + 10:(10 + VJ) * (bi + 1)]:
                j()

    @pl.when(i == 1)
    def _init2():
        cs = copies()
        wait(cs, 'wo')
        wait(cs, 'x1')

    def main(do_proj, do_out=True):
        slot = i % 2
        lane = jax.lax.broadcasted_iota(jnp.int32, (8, 128), 1)
        g = g_ref[slot]
        g_r = pltpu.roll(g, 64, 1)
        gsel = [jnp.where(lane < 64, g, g_r), jnp.where(lane < 64, g_r, g)]
        gates = (gsel, [1.0 - t for t in gsel])
        lane32 = jax.lax.broadcasted_iota(jnp.int32, (32, 128), 1)
        row40 = jax.lax.broadcasted_iota(jnp.int32, (40, 128), 0)
        lane40 = jax.lax.broadcasted_iota(jnp.int32, (40, 128), 1)
        selz = (lane40 < 64) == (row40 < 20)
        r64 = jax.lax.broadcasted_iota(jnp.int32, (64, 128), 0)
        c64 = jax.lax.broadcasted_iota(jnp.int32, (64, 128), 1) & 63
        low = r64 <= c64
        lane48 = jax.lax.broadcasted_iota(jnp.int32, (48, 128), 1)

        def masked_q(bi, p, hf):
            tl, off = PT[p]
            qt = pltpu.bitcast(q_ref[slot, bi, tl, 64 * hf:64 * hf + 64, :], jnp.int32)
            m0 = jnp.where((lane32 >= off) & (lane32 < off + 20), -1, 0)
            m1 = jnp.where((lane32 >= off + 20) & (lane32 < off + 40), -1, 0)
            return pltpu.bitcast(jnp.concatenate([qt & m0, qt & m1], axis=0), BF16), tl

        def qk(bi, p, hf):
            qm, tl = masked_q(bi, p, hf)
            k0 = pl.multiple_of(q0 + 64 * hf, 64)
            kk = (ka_ref, kb_ref)[bi][tl, pl.ds(k0, (RA, RB)[bi]), :]
            return jax.lax.dot_general(kk, qm, NT, preferred_element_type=F32)

        def cmax(a):
            return jnp.max(a.reshape(a.shape[0] // 8, 8, 128), axis=0)

        def smax_a(s, hf):
            hidx = 2 * i + hf
            st, sb = s[0:64], s[256:320]
            sg = jnp.where(low, sb, jnp.where(hidx >= 4, st, NEG))
            mids = [s[64 * c:64 * c + 64] for c in (1, 2, 3)]
            m8 = cmax(sg)
            for c in (1, 2, 3):
                m8 = jnp.maximum(m8, jnp.where(hidx + c >= 4, cmax(mids[c - 1]), NEG))
            m = jnp.max(m8, axis=0, keepdims=True)
            pg = jnp.exp2(sg - m)
            pm = [jnp.exp2(mids[c - 1] - jnp.where(hidx + c >= 4, m, -NEG)) for c in (1, 2, 3)]
            pt = jnp.where(low, 0.0, pg)
            pb = jnp.where(low, pg, 0.0)
            parts = [pt] + pm + [pb]
            if hf == 1:
                parts = [jnp.zeros((64, 128), F32)] + parts
            return jnp.concatenate(parts, axis=0).astype(BF16)

        def smax_b(s, hf):
            s = s + bias_ref[jnp.minimum(2 * i + hf, 1)]
            m = jnp.max(s, axis=0, keepdims=True)
            return jnp.exp2(s - m).astype(BF16)

        def pv_a(p, hf, pp):
            vv = cat1([va_ref[p, i], va_ref[p, i + 1], va_ref[p, i + 2]])
            return jnp.dot(vv[:, 0:pp.shape[0]], pp, preferred_element_type=F32)

        def pv_b(p, hf, pp):
            vcur = vb_ref[p, i + 1]
            if hf == 0:
                vv = jnp.where(lane48 < 16, pltpu.roll(vb_ref[p, i], 16, 1), pltpu.roll(vcur, 16, 1))
            else:
                vv = pltpu.roll(vcur, 80, 1)
            return jnp.dot(vv[:, 0:RB], pp, preferred_element_type=F32)

        def finish(res, gts):
            def nrm(r, gt):
                sm = r[40:48]
                rc = pltpu.reciprocal(sm, approx=True)
                rc = rc * (2.0 - sm * rc) * gt
                return (r[0:40].reshape(5, 8, 128) * rc[None]).reshape(40, 128)
            o0, o1 = nrm(res[0], gts[0]), nrm(res[1], gts[1])
            y = jnp.where(lane40 >= 64, o0, o1)
            z = jnp.where(lane40 < 64, o0, o1)
            return jnp.where(selz, z, pltpu.roll(y, 64, 1))

        tiles = [(p, hf) for p in range(NPAIR) for hf in range(2)]
        n = len(tiles)
        extra = (proj_jobs(i + 1) if do_proj else [])
        ojobs = out_jobs(1 - slot) if do_out else []
        D1, D2 = DEPTH
        nsteps = n + D1 + D2
        sv, pv_, res, fins = {}, {}, {}, {}
        def st_q(t):
            if t < n:
                sv[(0, t)] = qk(0, *tiles[t])
        def st_Q(t):
            if t < n:
                sv[(1, t)] = qk(1, *tiles[t])
        def st_e(t):
            if EOFF <= t < len(extra) + EOFF:
                extra[t - EOFF]()
            for k, oj in enumerate(ojobs):
                if t == nsteps - 1 - OSTEP * (len(ojobs) - 1 - k):
                    oj()
        def st_s(t):
            u = t - D1
            if 0 <= u < n:
                pv_[(0, u)] = smax_a(sv.pop((0, u)), tiles[u][1])
        def st_S(t):
            u = t - D1
            if 0 <= u < n:
                pv_[(1, u)] = smax_b(sv.pop((1, u)), tiles[u][1])
        def st_p(t):
            w = t - D1 - D2
            if 0 <= w < n:
                p, hf = tiles[w]
                res[(0, w)] = pv_a(p, hf, pv_.pop((0, w)))
        def st_P(t):
            w = t - D1 - D2
            if 0 <= w < n:
                p, hf = tiles[w]
                res[(1, w)] = pv_b(p, hf, pv_.pop((1, w)))
        def st_f(t):
            w = t - D1 - D2
            if 0 <= w < n:
                p, hf = tiles[w]
                if hf == 1:
                    for bi in range(2):
                        fins[(bi, p)] = finish([res.pop((bi, w - 1)), res.pop((bi, w))], gates[bi])
                        if p % 2 == 1:
                            ot_ref[slot, D * bi + 40 * (p - 1):D * bi + 40 * (p + 1), :] = jnp.concatenate(
                                [fins.pop((bi, p - 1)), fins.pop((bi, p))], axis=0)
        SCHED_FNS = dict(q=st_q, Q=st_Q, e=st_e, s=st_s, S=st_S, p=st_p, P=st_P, f=st_f)
        for t in range(nsteps):
            for ch in ORDER:
                SCHED_FNS[ch](t)

    @pl.when(i == 0)
    def _():
        main(True, False)

    @pl.when(jnp.logical_and(i > 0, i < NB - 1))
    def _():
        main(True)

    @pl.when(i == NB - 1)
    def _():
        main(False)

    @pl.when(i == NB)
    def _():
        for j in out_jobs((NB - 1) % 2):
            j()


@jax.jit
def pallas_gated_mix__sliding_block__sliding_local_dilated__prompt_kernel(
    A_x, A_wqkv, A_wo, B_x, B_wqkv, B_wo, gate_w):
    x = A_x.reshape(S, D)
    anyspec = pl.BlockSpec(memory_space=pl.ANY)
    out = pl.pallas_call(
        kernel,
        grid=(NB + 1,),
        in_specs=[anyspec] * 5 + [pl.BlockSpec((1, D), lambda i: (0, 0))],
        out_specs=pl.BlockSpec((TQ, D), lambda i: (jnp.maximum(i - 1, 0), 0)),
        out_shape=jax.ShapeDtypeStruct((S, D), BF16),
        scratch_shapes=[
            pltpu.VMEM((S, D), BF16),
            pltpu.VMEM((2, D, 3 * D), BF16),
            pltpu.VMEM((2, D, D), BF16),
            pltpu.VMEM((2, 5, D + 16, 128), BF16),
            pltpu.VMEM((10, D, 128), BF16),
            pltpu.VMEM((2, 2, 9, TQ, 128), BF16),
            pltpu.VMEM((9, PADA + S, 128), BF16),
            pltpu.VMEM((NPAIR, 2 + NB, 48, 128), BF16),
            pltpu.VMEM((9, PADB + S, 128), BF16),
            pltpu.VMEM((NPAIR, 1 + NB, 48, 128), BF16),
            pltpu.VMEM((2, 8, 128), F32),
            pltpu.VMEM((2, RB, 128), F32),
            pltpu.VMEM((2, 2 * D, TQ), F32),
            pltpu.SemaphoreType.DMA((7,)),
        ],
        compiler_params=pltpu.CompilerParams(dimension_semantics=("arbitrary",), vmem_limit_bytes=100 * 2**20),
    )(x, A_wqkv, A_wo, B_wqkv, B_wo, gate_w.reshape(1, D))
    return out.reshape(1, S, D)
```
